```python
import os as _os
_os.environ.setdefault("JAX_PLATFORMS", "cpu")
import jax
import jax.numpy as jnp

def _softmax(x, axis=-1):
    return jax.nn.softmax(x, axis=axis)
def _gelu(x):
    return jax.nn.gelu(x, approximate=True)
def _silu(x):
    return jax.nn.silu(x)
def _sigmoid(x):
    return jax.nn.sigmoid(x)
def _layernorm(x, axis=-1, eps=1e-5):
    m = jnp.mean(x, axis=axis, keepdims=True)
    v = jnp.var(x, axis=axis, keepdims=True)
    return (x - m) / jnp.sqrt(v + eps)
def _scatter_add(tgt, idx, src, axis=0):
    return tgt.at[idx].add(src)
def _segment_sum(src, seg, n):
    return jax.ops.segment_sum(src, seg, n)
class _Rng:
    def __init__(self, key):
        self._k = key
    def _next(self):
        self._k, sub = jax.random.split(self._k)
        return sub
    def normal(self, shape):
        return jax.random.normal(self._next(), shape, dtype=jnp.bfloat16)
    def randint(self, lo, hi, shape):
        return jax.random.randint(self._next(), shape, lo, hi, dtype=jnp.int32)
    def uniform(self, shape, lo=0.0, hi=1.0):
        return jax.random.uniform(self._next(), shape, jnp.bfloat16, lo, hi)
    def permutation(self, n):
        return jax.random.permutation(self._next(), n)


kernel_name = 'interleave_layers__gqa_block_cached__dense_activation_silu__decode'

def setup_inputs():
    _rng = _Rng(jax.random.key(int.from_bytes(__import__("os").urandom(4), "little")))
    _w = (lambda a: (lambda t: t.astype(jnp.bfloat16) if jnp.issubdtype(t.dtype, jnp.floating) else t)(jnp.asarray(a)))
    def _A_setup():
        B, Sq, D = 2, 1, 512
        Hq, Hkv, Sk, Dh = 32, 8, 8192, 128
        assert Hq % Hkv == 0, (Hq, Hkv)
        return {
            "x": _w((lambda *s: _rng.normal(s) * 0.1)(B, Sq, D)),
            "k_cache": _w((lambda *s: _rng.normal(s) * 0.8)(B, Hkv, Sk, Dh)),
            "v_cache": _w((lambda *s: _rng.normal(s) * 1.6)(B, Hkv, Sk, Dh)),
            "wq": _w((lambda *s: _rng.normal(s) * 0.8)(D, Hq * Dh) * (D ** -0.5)),
            "wo": _w((lambda *s: _rng.normal(s) * 1.6)(Hq * Dh, D) * ((Hq * Dh) ** -0.5)),
        }
    _A_in = _A_setup()

    def _B_setup():
        B, S, D, F = 2, 1, 512, 1792
        return {
            "x": _w((lambda *s: _rng.normal(s) * 0.1)(B, S, D)),
            "w1": _w((lambda *s: _rng.normal(s) * 0.4)(D, F) * (D ** -0.5)),
            "w2": _w((lambda *s: _rng.normal(s) * 0.4)(F, D) * (F ** -0.5)),
        }
    _B_in = _B_setup()

    return {
        "A_x": _A_in["x"],
        "A_k_cache": _A_in["k_cache"],
        "A_v_cache": _A_in["v_cache"],
        "A_wq": _A_in["wq"],
        "A_wo": _A_in["wo"],
        "B_x": _B_in["x"],
        "B_w1": _B_in["w1"],
        "B_w2": _B_in["w2"],
    }

def reference(A_x, A_k_cache, A_v_cache, A_wq, A_wo, B_x, B_w1, B_w2):
    def _A_ref(x, k_cache, v_cache, wq, wo):
        B, Sq, D = x.shape
        Hq, Dh = 32, 128
        Hkv = k_cache.shape[1]
        rep = Hq // Hkv
        q = (lambda x, *d: x.transpose(*d))((x @ wq).reshape(B, Sq, Hq, Dh), 0, 2, 1, 3)
        k = jnp.repeat(k_cache, rep, axis=1)
        v = jnp.repeat(v_cache, rep, axis=1)
        scores = jnp.einsum("bhqd,bhkd->bhqk", q, k) * (Dh ** -0.5)
        p = _softmax(scores, axis=-1)
        o = jnp.einsum("bhqk,bhkd->bhqd", p, v)
        return (lambda x, *d: x.transpose(*d))(o, 0, 2, 1, 3).reshape(B, Sq, Hq * Dh) @ wo

    def _B_ref(x, w1, w2):
        h = jnp.einsum("bsd,df->bsf", x, w1)
        h = _silu(h)
        out = jnp.einsum("bsf,fd->bsd", h, w2)
        return out

    x = A_x
    x = x + _A_ref(_layernorm(x, axis=-1), A_k_cache, A_v_cache, A_wq, A_wo)
    x = x + _B_ref(_layernorm(x, axis=-1), B_w1, B_w2)
    x = x + _A_ref(_layernorm(x, axis=-1), A_k_cache, A_v_cache, A_wq, A_wo)
    x = x + _B_ref(_layernorm(x, axis=-1), B_w1, B_w2)
    return x
```

```python
import functools
import jax
import jax.numpy as jnp
from jax import lax
from jax.experimental import pallas as pl
from jax.experimental.pallas import tpu as pltpu

B, D, HKV, REP, DH, S, F = 2, 512, 8, 4, 128, 8192, 1792
G = REP * DH
H2 = S // 2
NJ = H2 // DH
SCALE = DH ** -0.5
f32, bf16, u32 = jnp.float32, jnp.bfloat16, jnp.uint32
NT = B * HKV
NC = 4
NODMA = False
NAME = "v4"
ALL = slice(None)


def _ld(ref, *idx):
    return pltpu.bitcast(ref[idx], bf16)


def _dot(a, b):
    return jnp.dot(a, b, preferred_element_type=f32)


def _center(x):
    d = x - jnp.mean(x, axis=-1, keepdims=True)
    r = lax.rsqrt(jnp.mean(d * d, axis=-1, keepdims=True) + 1e-5)
    return d.astype(bf16), r


def kernel(x_hbm, k_hbm, v_hbm, wq_hbm, wo_hbm, w1_hbm, w2_hbm, o_hbm,
           xb, kb0, kb1, vb, wq, wo, w1, w2, ob, s_a, s_b, sem_k, sem_v, sem_w):
    k32, v32 = k_hbm.bitcast(u32), v_hbm.bitcast(u32)
    kbs = (kb0, kb1)

    def cp_k(b, g):
        return pltpu.make_async_copy(k32.at[b * HKV + g], kbs[b].at[g], sem_k.at[g % 4])

    def cp_v(t):
        return pltpu.make_async_copy(v32.at[t], vb.at[t], sem_v.at[t % 4])

    def cp_vc(c):
        rows = pl.ds(c * (H2 // NC), H2 // NC)
        return pltpu.make_async_copy(v32.at[NT - 1, rows], vb.at[NT - 1, rows], sem_k.at[c])

    cp_x = pltpu.make_async_copy(x_hbm, xb, sem_w.at[0])
    cp_wq = pltpu.make_async_copy(wq_hbm.bitcast(u32), wq, sem_w.at[1])
    cp_wo = pltpu.make_async_copy(wo_hbm.bitcast(u32), wo, sem_w.at[2])
    cp_w1 = pltpu.make_async_copy(w1_hbm.bitcast(u32), w1, sem_w.at[1])
    cp_w2 = pltpu.make_async_copy(w2_hbm.bitcast(u32), w2, sem_w.at[0])
    cp_o = pltpu.make_async_copy(ob, o_hbm, sem_w.at[0])

    def start(c):
        if not NODMA:
            c.start()

    def wait(c):
        if not NODMA:
            c.wait()

    start(cp_wq)
    cp_x.start()
    start(cp_k(0, 0))
    start(cp_k(0, 1))
    start(cp_v(0))

    row = lax.broadcasted_iota(jnp.int32, (8, DH), 0)
    head = row % REP
    top = row < REP

    def q_for(xn, g):
        d, r = xn
        qf = _dot(d, _ld(wq, ALL, pl.ds(pl.multiple_of(g * G, G), G)))
        q = qf[:, 0:DH]
        for j in range(1, REP):
            q = jnp.where(head == j, qf[:, j * DH:(j + 1) * DH], q)
        q = q * r
        return jnp.where(top, q, 0.0).astype(bf16), jnp.where(top, 0.0, q).astype(bf16)

    def transpose_k(b, g):
        for j in range(S // DH):
            sl = pl.ds(j * 64, 64)
            kbs[b][g, sl, :] = pltpu.bitcast(_ld(kbs[b], g, sl, ALL).T, u32)

    def scores(q, b, g, s_ref):
        qa, qb = q
        m = None
        for j in range(NJ):
            s = (_dot(qa, _ld(kbs[b], g, pl.ds(j * 64, 64), ALL))
                 + _dot(qb, _ld(kbs[b], g, pl.ds(H2 // 2 + j * 64, 64), ALL)))
            s_ref[:, j * DH:(j + 1) * DH] = s
            m = s if m is None else jnp.maximum(m, s)
        m = jnp.maximum(m, pltpu.roll(m, REP, 0))
        return jnp.broadcast_to(jnp.max(m, axis=-1, keepdims=True), (8, DH))

    def probs(m, s_ref):
        p = [jnp.exp((s_ref[:, j * DH:(j + 1) * DH] - m) * SCALE) for j in range(NJ)]
        l = functools.reduce(jnp.add, p)
        l = l + pltpu.roll(l, REP, 0)
        l = jnp.sum(l, axis=-1, keepdims=True)
        return jnp.concatenate(p, axis=1).astype(bf16), 1.0 / l

    def pv(p, t):
        oa = _dot(p, _ld(vb, t, pl.ds(0, H2 // 2), ALL))
        ob_ = _dot(p, _ld(vb, t, pl.ds(H2 // 2, H2 // 2), ALL))
        return oa, ob_

    def normalize(oa, ob_, rl):
        o = jnp.where(top, oa, ob_)
        return (o + pltpu.roll(o, REP, 0)) * rl

    def out_proj(o, g, acc):
        lhs = jnp.concatenate([jnp.where(row == j, o, 0.0) for j in range(REP)], axis=1).astype(bf16)
        return acc + _dot(lhs, _ld(wo, pl.ds(pl.multiple_of(g * (G // 2), G // 2), G // 2), ALL))

    def attend(m, s_ref, t, g, acc):
        p, rl = probs(m, s_ref)
        return out_proj(normalize(*pv(p, t), rl), g, acc)

    def finish(x, acc):
        x = x + jnp.sum(acc, axis=0, keepdims=True)
        d, r = _center(x)
        h = _dot(d, _ld(w1, ALL, ALL)) * r
        h = h * jax.nn.sigmoid(h)
        return x + _dot(h.astype(bf16), _ld(w2, ALL, ALL))

    def layer2(xn, b, heads, acc):
        n = len(heads)
        bufs = (s_a, s_b)
        q = q_for(xn, heads[0])
        qn = q_for(xn, heads[1]) if n > 1 else None
        m = scores(q, b, heads[0], bufs[0])
        o = None
        for i in range(n):
            q, qn = qn, (q_for(xn, heads[i + 2]) if i + 2 < n else None)
            mn = scores(q, b, heads[i + 1], bufs[(i + 1) % 2]) if i + 1 < n else None
            p, rl = probs(m, bufs[i % 2])
            on = normalize(*pv(p, b * HKV + heads[i]), rl)
            if o is not None:
                acc = out_proj(o, heads[i - 1], acc)
            m, o = mn, on
        return out_proj(o, heads[n - 1], acc)

    cp_x.wait()
    xx = xb[...].astype(f32)
    x0 = jnp.broadcast_to(xx[0:1], (8, D))
    x1 = jnp.broadcast_to(xx[1:2], (8, D))
    xn0 = _center(x0)
    xn1 = _center(x1)
    zero = jnp.zeros((8, D), f32)
    wait(cp_wq)
    start(cp_wo)
    wait(cp_k(0, 0))
    start(cp_k(0, 2))
    transpose_k(0, 0)

    def ph1(g, acc):
        m = scores(q_for(xn0, g), 0, g, s_a)
        wait(cp_k(0, g + 1))
        start(cp_v(g + 1))
        transpose_k(0, g + 1)
        wait(cp_v(g))

        @pl.when(g + 3 < HKV)
        def _():
            start(cp_k(0, g + 3))

        @pl.when(g + 3 >= HKV)
        def _():
            start(cp_k(1, g + 3 - HKV))

        @pl.when(g == 0)
        def _():
            wait(cp_wo)

        @pl.when(g == 1)
        def _():
            start(cp_w1)

        @pl.when(g == 3)
        def _():
            start(cp_w2)

        return attend(m, s_a, g, g, acc)

    acc = lax.fori_loop(0, HKV - 1, ph1, zero)
    g = HKV - 1
    m = scores(q_for(xn0, g), 0, g, s_a)
    wait(cp_k(1, 0))
    start(cp_v(g + 1))
    transpose_k(1, 0)
    wait(cp_v(g))
    start(cp_k(1, 2))
    acc = attend(m, s_a, g, g, acc)
    wait(cp_w1)
    wait(cp_w2)
    x0 = finish(x0, acc)
    xn0 = _center(x0)
    a0 = layer2(xn0, 0, [0, 1], zero)

    def ph2(g, accs):
        a0, a1 = accs
        t = HKV + g
        m = scores(q_for(xn1, g), 1, g, s_a)
        wait(cp_k(1, g + 1))
        start(cp_v(t + 1))
        transpose_k(1, g + 1)
        m0 = scores(q_for(xn0, g + 2), 0, g + 2, s_b)
        a0 = attend(m0, s_b, g + 2, g + 2, a0)
        wait(cp_v(t))

        @pl.when(g + 3 < HKV)
        def _():
            start(cp_k(1, g + 3))

        return a0, attend(m, s_a, t, g, a1)

    a0, a1 = lax.fori_loop(0, HKV - 2, ph2, (a0, zero))
    g = HKV - 2
    m = scores(q_for(xn1, g), 1, g, s_a)
    wait(cp_k(1, g + 1))
    start(cp_vc(0))
    transpose_k(1, g + 1)
    x0 = finish(x0, a0)
    start(cp_vc(1))
    start(cp_vc(2))
    wait(cp_v(HKV + g))
    start(cp_vc(3))
    mn = scores(q_for(xn1, g + 1), 1, g + 1, s_b)
    a1 = attend(m, s_a, HKV + g, g, a1)
    p, rl = probs(mn, s_b)
    parts = []
    w = H2 // NC
    for c in range(NC):
        wait(cp_vc(c))
        half, off = divmod(c * 2 * w, H2)
        parts.append(_dot(p[:, off:off + 2 * w], _ld(vb, NT - 1, pl.ds(c * w, w), ALL)))
    oa = functools.reduce(jnp.add, parts[:NC // 2])
    ob_ = functools.reduce(jnp.add, parts[NC // 2:])
    a1 = out_proj(normalize(oa, ob_, rl), g + 1, a1)
    x1 = finish(x1, a1)
    x1 = finish(x1, layer2(_center(x1), 1, list(range(HKV)), zero))
    r8 = lax.broadcasted_iota(jnp.int32, (8, D), 0)
    ob[...] = jnp.where(r8 == 0, x0, x1)[0:2].astype(bf16)
    cp_o.start()
    cp_o.wait()


@jax.jit
def pallas_interleave_layers__gqa_block_cached__dense_activation_silu__decode_kernel(A_x, A_k_cache, A_v_cache, A_wq, A_wo, B_x, B_w1, B_w2):
    anyspec = pl.BlockSpec(memory_space=pl.ANY)
    out = pl.pallas_call(
        kernel,
        out_shape=jax.ShapeDtypeStruct((B, D), A_x.dtype),
        in_specs=[anyspec] * 7,
        out_specs=anyspec,
        scratch_shapes=[
            pltpu.VMEM((B, D), bf16),
            pltpu.VMEM((HKV, S // 2, DH), u32),
            pltpu.VMEM((HKV, S // 2, DH), u32),
            pltpu.VMEM((NT, S // 2, DH), u32),
            pltpu.VMEM((D // 2, HKV * G), u32),
            pltpu.VMEM((HKV * G // 2, D), u32),
            pltpu.VMEM((D // 2, F), u32),
            pltpu.VMEM((F // 2, D), u32),
            pltpu.VMEM((B, D), bf16),
            pltpu.VMEM((8, H2), f32),
            pltpu.VMEM((8, H2), f32),
            pltpu.SemaphoreType.DMA((4,)),
            pltpu.SemaphoreType.DMA((4,)),
            pltpu.SemaphoreType.DMA((3,)),
        ],
        compiler_params=pltpu.CompilerParams(vmem_limit_bytes=110 * 1024 * 1024),
        name=NAME,
    )(A_x.reshape(B, D), A_k_cache.reshape(NT, S, DH), A_v_cache.reshape(NT, S, DH),
      A_wq, A_wo, B_w1, B_w2)
    return out.reshape(A_x.shape)
```

```python
import functools

import jax
import jax.numpy as jnp
from jax import lax
from jax.experimental import pallas as pl
from jax.experimental.pallas import tpu as pltpu

B, D, HKV, REP, DH, S, F = 2, 512, 8, 4, 128, 8192, 1792
G = REP * DH
H2 = S // 2
NJ = H2 // DH
ND = D // DH
NF = F // DH
NT = B * HKV
NC = 4
CW = S // NC
W1_VPU, W2_VPU = 2, 3
SCALE = DH ** -0.5
f32, bf16, u32 = jnp.float32, jnp.bfloat16, jnp.uint32
ALL = slice(None)


def _ld(ref, *idx):
    return pltpu.bitcast(ref[idx], bf16)


def _pack(x):
    return pltpu.bitcast(x, u32)


def _dot(a, b):
    return jnp.dot(a, b, preferred_element_type=f32)


def _sum(xs):
    return functools.reduce(jnp.add, xs)


def _tiles(x):
    return [x[:, i:i + DH] for i in range(0, x.shape[1], DH)]


def _after(x, dep):
    b = pltpu.bitcast(dep, u32)
    z = (b >> 31) & ((~b) >> 31)
    z = jnp.concatenate([z] * (x.shape[0] // 8), axis=0)
    return pltpu.bitcast(pltpu.bitcast(x, u32) | z, f32)


def _store_columns(ref, rows):
    for i, r in enumerate(rows):
        ref[pl.ds(i * DH, DH), :] = jnp.broadcast_to(r, (DH, DH)).T


def _vpu_rows(accs, w_ref, r16, c0, col):
    for n in range(len(accs)):
        cols = pl.ds(c0 + n * DH, DH)
        if w_ref.dtype == u32:
            w = _ld(w_ref, pl.ds(r16 * 8, 8), cols)
        else:
            w = w_ref[pl.ds(r16 * 16, 16), cols]
        w = w.astype(f32) * col
        w = w[0:8] + w[8:16]
        accs[n] = w if accs[n] is None else accs[n] + w


def _layernorm(x, mean=None):
    if mean is None:
        mean = jnp.mean(x, axis=-1, keepdims=True)
    d = x - mean
    r = lax.rsqrt(jnp.mean(d * d, axis=-1, keepdims=True) + 1e-5)
    return d.astype(bf16), r


def _silu(h):
    return h * jax.nn.sigmoid(h)


def _kernel(x_hbm, k_hbm, v_hbm, wq_hbm, wo_hbm, w1_hbm, w2_hbm, o_hbm,
            xb, kraw, kt0, kt1, vb, wq, wo, wq32, wo32, w1, w2, ob, s_a, s_b, xcol, ocol, hcol, wsum,
            sem_k, sem_v, sem_w):
    kts = (kt0, kt1)
    v32 = kt0

    def cp_k(b, g):
        return pltpu.make_async_copy(k_hbm.at[b * HKV + g], kraw.at[g % 2], sem_k.at[g % 2])

    def cp_v(t):
        return pltpu.make_async_copy(v_hbm.at[t], vb.at[t], sem_v.at[t % 2])

    def cp_v_last(c):
        rows = pl.ds(c * CW, CW)
        sem = sem_k.at[c] if c < 2 else sem_w.at[c - 1]
        return pltpu.make_async_copy(v_hbm.at[NT - 1, rows], vb.at[NT - 1, rows], sem)

    cp_x = pltpu.make_async_copy(x_hbm, xb, sem_w.at[0])
    cp_wq = pltpu.make_async_copy(wq_hbm, wq, sem_w.at[1])
    cp_wo = pltpu.make_async_copy(wo_hbm, wo, sem_w.at[2])
    cp_w1 = pltpu.make_async_copy(w1_hbm, w1, sem_w.at[1])
    cp_w2 = pltpu.make_async_copy(w2_hbm, w2, sem_w.at[0])
    cp_o = pltpu.make_async_copy(ob, o_hbm, sem_w.at[0])

    cp_wq.start()
    cp_x.start()
    cp_k(0, 0).start()
    cp_k(0, 1).start()
    cp_v(0).start()

    row = lax.broadcasted_iota(jnp.int32, (8, DH), 0)
    head = row % REP
    top = row < REP

    def by_head(tiles):
        q = tiles[0]
        for h in range(1, REP):
            q = jnp.where(head == h, tiles[h], q)
        return q

    def split(q):
        return jnp.where(top, q, 0.0).astype(bf16), jnp.where(top, 0.0, q).astype(bf16)

    def q_from(xn, w):
        d, r = xn
        return split(by_head(_tiles(_dot(d, w))) * r)

    def q_proj(xn, g, keep=False):
        cols = pl.ds(pl.multiple_of(g * G, G), G)
        w = wq[:, cols]
        if keep:
            wq32[:, cols] = _pack(w)
        return q_from(xn, w)

    def transpose_k(b, g):
        for j in range(S // DH):
            kts[b][g, pl.ds(j * 64, 64), :] = _pack(kraw[g % 2, pl.ds(j * DH, DH), :].T)

    def scores(q, b, g, s_ref, each=None):
        m = None
        for j in range(NJ):
            s = (_dot(q[0], _ld(kts[b], g, pl.ds(j * 64, 64), ALL))
                 + _dot(q[1], _ld(kts[b], g, pl.ds(H2 // 2 + j * 64, 64), ALL)))
            s_ref[:, j * DH:(j + 1) * DH] = s
            m = s if m is None else jnp.maximum(m, s)
            if each is not None:
                each(j, s)
        m = jnp.maximum(m, pltpu.roll(m, REP, 0))
        return jnp.broadcast_to(jnp.max(m, axis=-1, keepdims=True), (8, DH))

    def exps(m, s_ref):
        return [jnp.exp((s_ref[:, j * DH:(j + 1) * DH] - m) * SCALE) for j in range(NJ)]

    def inv_total(p):
        l = _sum(p)
        l = l + pltpu.roll(l, REP, 0)
        return 1.0 / jnp.sum(l, axis=-1, keepdims=True)

    def normalize(o_lo, o_hi, rl):
        o = jnp.where(top, o_lo, o_hi)
        return (o + pltpu.roll(o, REP, 0)) * rl

    def v_rows(b, g, start, n, keep=False):
        v = vb[b * HKV + g, pl.ds(start, n), :]
        if keep:
            v32[g, pl.ds(start // 2, n // 2), :] = _pack(v)
        return v

    def v_rows_packed(g, start, n):
        return _ld(v32, g, pl.ds(start // 2, n // 2), ALL)

    def attend(m, s_ref, v):
        p = exps(m, s_ref)
        rl = inv_total(p)
        p = jnp.concatenate(p, axis=1).astype(bf16)
        return normalize(_dot(p, v(0, H2)), _dot(p, v(H2, H2)), rl)

    def out_proj(o, g, keep=False):
        lhs = jnp.concatenate([jnp.where(row == h, o, 0.0) for h in range(REP)], axis=1)
        w = wo[pl.ds(pl.multiple_of(g * G, G), G), :]
        if keep:
            wo32[pl.ds(pl.multiple_of(g * (G // 2), G // 2), G // 2), :] = _pack(w)
        return _dot(lhs.astype(bf16), w)

    def ffn(x):
        d, r = _layernorm(x)
        h = _silu(_dot(d, w1[...]) * r)
        return x + _dot(h.astype(bf16), w2[...])

    def last_head_and_ffn(x, acc, o):
        x = x + jnp.sum(acc, axis=0, keepdims=True)
        t = jnp.where(top, o.astype(bf16).astype(f32) * wsum[:, F:F + DH], 0.0)
        t = _sum(_tiles(x)) + jnp.sum(t, axis=0, keepdims=True)
        mean = jnp.sum(t, axis=-1, keepdims=True) * (1.0 / D)
        flat = jnp.concatenate(
            [jnp.broadcast_to(o[h:h + 1], (8, DH)) for h in range(REP)], axis=1)
        x = x + _dot(flat.astype(bf16), wo[pl.ds((HKV - 1) * G, G), :])
        d, r = _layernorm(x, mean)

        def hidden(h):
            return _tiles(_silu(h * r).astype(bf16).astype(f32))

        hs, rounds = [], []
        n_mxu = NF - W1_VPU
        for c in range(0, n_mxu, 4):
            ys = [_dot(d[:, k * DH:(k + 1) * DH],
                       w1[pl.ds(k * DH, DH), pl.ds(c * DH, min(4, n_mxu - c) * DH)])
                  for k in range(ND)]
            rounds += [y[:, 0:DH] for y in ys]
            hs += hidden(_sum(ys))
        df = d.astype(f32)
        _store_columns(xcol, [df[0:1, c * DH:(c + 1) * DH] for c in range(ND)])
        h_acc = [None] * W1_VPU
        n1, r1 = D // 16, len(rounds)
        for i in range(n1):
            col = _after(xcol[pl.ds(i * 16, 16), :], rounds[i * r1 // n1])
            _vpu_rows(h_acc, w1, i, n_mxu * DH, col)
        hs += hidden(jnp.sum(jnp.concatenate(h_acc, axis=1), axis=0, keepdims=True))

        t = _sum(_tiles(x))
        for c in range(NF):
            t = t + hs[c] * wsum[:, c * DH:(c + 1) * DH]
        ys = [_dot(hs[c].astype(bf16), w2[pl.ds(c * DH, DH), :])
              for c in range(W2_VPU, NF)]
        rounds += [y[:, 0:DH] for y in ys]
        _store_columns(hcol, [hs[c][0:1] for c in range(W2_VPU)])
        y_acc = [None] * ND
        n2 = W2_VPU * DH // 16
        for i in range(n2):
            col = _after(hcol[pl.ds(i * 16, 16), :], rounds[r1 - 1 + i * (len(ys) - 2) // n2])
            _vpu_rows(y_acc, w2, i, 0, col)
        x = x + jnp.sum(jnp.concatenate(y_acc, axis=1), axis=0, keepdims=True)
        return x + _sum(ys), jnp.sum(t, axis=-1, keepdims=True) * (1.0 / D)

    def resident_attention(xn):
        d, r = xn
        bufs = (s_a, s_b)
        accs = [None] * ND
        df = d.astype(f32)
        _store_columns(xcol, [df[0:1, c * DH:(c + 1) * DH] for c in range(ND)])

        def scores_and_next_q(q, g, s_ref):
            q_acc = [None] * REP
            m = scores(q, 1, g, s_ref, lambda j, s: _vpu_rows(
                q_acc, wq32, j, (g + 1) * G, _after(xcol[pl.ds(j * 16, 16), :], s)))
            q = by_head([jnp.broadcast_to(jnp.sum(a, axis=0, keepdims=True), (8, DH))
                         for a in q_acc])
            return m, split(q * r)

        def wo_rows(g, j, dep):
            _vpu_rows(accs, wo32, g * (G // 16) + j, 0, _after(ocol[pl.ds(j * 16, 16), :], dep))

        def attend_and_prev_wo(m, s_ref, g):
            p = exps(m, s_ref)
            o_lo = o_hi = None
            for j in range(NJ):
                pj = p[j].astype(bf16)
                lo = _dot(pj, v_rows_packed(g, j * DH, DH))
                hi = _dot(pj, v_rows_packed(g, H2 + j * DH, DH))
                o_lo, o_hi = (lo, hi) if o_lo is None else (o_lo + lo, o_hi + hi)
                wo_rows(g - 1, j, o_lo)
            return normalize(o_lo, o_hi, inv_total(p))

        q0, q1 = (q_from(xn, _ld(wq32, ALL, pl.ds(g * G, G))) for g in range(2))
        m0 = scores(q0, 1, 0, s_a)
        m, q = scores_and_next_q(q1, 1, s_b)
        o = attend(m0, s_a, functools.partial(v_rows_packed, 0))
        for i in range(1, HKV):
            cur, nxt = bufs[i % 2], bufs[(i + 1) % 2]
            o = o.astype(bf16).astype(f32)
            _store_columns(ocol, [o[h:h + 1] for h in range(REP)])
            if i + 2 < HKV:
                m_next, q = scores_and_next_q(q, i + 1, nxt)
                o = attend_and_prev_wo(m, cur, i)
                m = _after(m_next, _sum(accs))
            elif i + 1 < HKV:
                m_next = scores(q, 1, i + 1, nxt, functools.partial(wo_rows, i - 1))
                o, m = attend(m, cur, functools.partial(v_rows_packed, i)), m_next
            else:
                o = attend_and_prev_wo(m, cur, i)
        return jnp.concatenate(accs, axis=1), o

    cp_x.wait()
    xx = xb[...].astype(f32)
    x0 = jnp.broadcast_to(xx[0:1], (8, D))
    x1 = jnp.broadcast_to(xx[1:2], (8, D))
    xn0 = _layernorm(x0)
    xn1 = _layernorm(x1)
    zero = jnp.zeros((8, D), f32)
    cp_wq.wait()
    cp_wo.start()
    cp_k(0, 0).wait()
    transpose_k(0, 0)
    cp_k(0, 2).start()

    def phase1(g, acc):
        m = scores(q_proj(xn0, g), 0, g, s_a)
        cp_k(0, g + 1).wait()
        cp_v(g + 1).start()
        transpose_k(0, g + 1)
        cp_v(g).wait()

        @pl.when(g + 3 < HKV)
        def _():
            cp_k(0, g + 3).start()

        @pl.when(g + 3 >= HKV)
        def _():
            cp_k(1, g + 3 - HKV).start()

        @pl.when(g == 0)
        def _():
            cp_wo.wait()

        @pl.when(g == 1)
        def _():
            cp_w1.start()

        @pl.when(g == 3)
        def _():
            cp_w2.start()

        return acc + out_proj(attend(m, s_a, functools.partial(v_rows, 0, g)), g)

    acc = lax.fori_loop(0, HKV - 1, phase1, zero)
    g = HKV - 1
    m = scores(q_proj(xn0, g), 0, g, s_a)
    cp_k(1, 0).wait()
    cp_v(HKV).start()
    cp_w1.wait()
    cp_w2.wait()
    transpose_k(1, 0)
    ones = jnp.ones((8, D), bf16)
    nt = (((1,), (1,)), ((), ()))
    wsum[:, 0:F] = lax.dot_general(ones, w2[...], nt, preferred_element_type=f32)
    wsum[:, F:F + DH] = by_head(_tiles(lax.dot_general(
        ones, wo[pl.ds(g * G, G), :], nt, preferred_element_type=f32)))
    cp_v(g).wait()
    cp_k(1, 2).start()
    acc = acc + out_proj(attend(m, s_a, functools.partial(v_rows, 0, g)), g)
    x0 = ffn(x0 + jnp.sum(acc, axis=0, keepdims=True))

    xn0 = _layernorm(x0)
    q0, q1 = q_proj(xn0, 0), q_proj(xn0, 1)
    m0 = scores(q0, 0, 0, s_a)
    m1 = scores(q1, 0, 1, s_b)
    a0 = (out_proj(attend(m0, s_a, functools.partial(v_rows, 0, 0)), 0)
          + out_proj(attend(m1, s_b, functools.partial(v_rows, 0, 1)), 1))

    def phase2(g, accs):
        a0, a1 = accs
        t = HKV + g
        m = scores(q_proj(xn1, g, keep=True), 1, g, s_a)
        cp_k(1, g + 1).wait()
        cp_v(t + 1).start()
        transpose_k(1, g + 1)
        m0 = scores(q_proj(xn0, g + 2), 0, g + 2, s_b)
        a0 = a0 + out_proj(attend(m0, s_b, functools.partial(v_rows, 0, g + 2)), g + 2)
        cp_v(t).wait()

        @pl.when(g + 3 < HKV)
        def _():
            cp_k(1, g + 3).start()

        o = attend(m, s_a, functools.partial(v_rows, 1, g, keep=True))
        return a0, a1 + out_proj(o, g, keep=True)

    a0, a1 = lax.fori_loop(0, HKV - 2, phase2, (a0, zero))
    g = HKV - 2
    m = scores(q_proj(xn1, g, keep=True), 1, g, s_a)
    cp_k(1, g + 1).wait()
    cp_v_last(0).start()
    transpose_k(1, g + 1)
    x0 = ffn(x0 + jnp.sum(a0, axis=0, keepdims=True))
    cp_v_last(1).start()
    cp_v_last(2).start()
    cp_v(HKV + g).wait()
    cp_v_last(3).start()
    m_last = scores(q_proj(xn1, g + 1, keep=True), 1, g + 1, s_b)
    o = attend(m, s_a, functools.partial(v_rows, 1, g, keep=True))
    a1 = a1 + out_proj(o, g, keep=True)
    p = exps(m_last, s_b)
    rl = inv_total(p)
    p = jnp.concatenate(p, axis=1).astype(bf16)
    parts = []
    for c in range(NC):
        cp_v_last(c).wait()
        off = c * CW % H2
        parts.append(_dot(p[:, off:off + CW], v_rows(1, HKV - 1, c * CW, CW, keep=True)))
    o = normalize(_sum(parts[:NC // 2]), _sum(parts[NC // 2:]), rl)

    x1, mean = last_head_and_ffn(x1, a1, o)
    a1, o = resident_attention(_layernorm(x1, mean))
    x1, _ = last_head_and_ffn(x1, a1, o)

    r8 = lax.broadcasted_iota(jnp.int32, (8, D), 0)
    ob[...] = jnp.where(r8 == 0, x0, x1)[0:B].astype(bf16)
    cp_o.start()
    cp_o.wait()


@jax.jit
def pallas_interleave_layers__gqa_block_cached__dense_activation_silu__decode_kernel(
    A_x: jax.Array,
    A_k_cache: jax.Array,
    A_v_cache: jax.Array,
    A_wq: jax.Array,
    A_wo: jax.Array,
    B_x: jax.Array,
    B_w1: jax.Array,
    B_w2: jax.Array,
):
    hbm = pl.BlockSpec(memory_space=pl.ANY)
    out = pl.pallas_call(
        _kernel,
        out_shape=jax.ShapeDtypeStruct((B, D), A_x.dtype),
        in_specs=[hbm] * 7,
        out_specs=hbm,
        scratch_shapes=[
            pltpu.VMEM((B, D), bf16),
            pltpu.VMEM((2, S, DH), bf16),
            pltpu.VMEM((HKV, S // 2, DH), u32),
            pltpu.VMEM((HKV, S // 2, DH), u32),
            pltpu.VMEM((NT, S, DH), bf16),
            pltpu.VMEM((D, HKV * G), bf16),
            pltpu.VMEM((HKV * G, D), bf16),
            pltpu.VMEM((D // 2, HKV * G), u32),
            pltpu.VMEM((HKV * G // 2, D), u32),
            pltpu.VMEM((D, F), bf16),
            pltpu.VMEM((F, D), bf16),
            pltpu.VMEM((B, D), bf16),
            pltpu.VMEM((8, H2), f32),
            pltpu.VMEM((8, H2), f32),
            pltpu.VMEM((D, DH), f32),
            pltpu.VMEM((G, DH), f32),
            pltpu.VMEM((W2_VPU * DH, DH), f32),
            pltpu.VMEM((8, F + DH), f32),
            pltpu.SemaphoreType.DMA((2,)),
            pltpu.SemaphoreType.DMA((2,)),
            pltpu.SemaphoreType.DMA((3,)),
        ],
        compiler_params=pltpu.CompilerParams(vmem_limit_bytes=110 * 1024 * 1024),
    )(A_x.reshape(B, D), A_k_cache.reshape(NT, S, DH), A_v_cache.reshape(NT, S, DH),
      A_wq, A_wo, B_w1, B_w2)
    return out.reshape(A_x.shape)
```
